```python
import os as _os
_os.environ.setdefault("JAX_PLATFORMS", "cpu")
import jax
import jax.numpy as jnp

def _softmax(x, axis=-1):
    return jax.nn.softmax(x, axis=axis)
def _gelu(x):
    return jax.nn.gelu(x, approximate=True)
def _silu(x):
    return jax.nn.silu(x)
def _sigmoid(x):
    return jax.nn.sigmoid(x)
def _layernorm(x, axis=-1, eps=1e-5):
    m = jnp.mean(x, axis=axis, keepdims=True)
    v = jnp.var(x, axis=axis, keepdims=True)
    return (x - m) / jnp.sqrt(v + eps)
def _scatter_add(tgt, idx, src, axis=0):
    return tgt.at[idx].add(src)
def _segment_sum(src, seg, n):
    return jax.ops.segment_sum(src, seg, n)
class _Rng:
    def __init__(self, key):
        self._k = key
    def _next(self):
        self._k, sub = jax.random.split(self._k)
        return sub
    def normal(self, shape):
        return jax.random.normal(self._next(), shape, dtype=jnp.bfloat16)
    def randint(self, lo, hi, shape):
        return jax.random.randint(self._next(), shape, lo, hi, dtype=jnp.int32)
    def uniform(self, shape, lo=0.0, hi=1.0):
        return jax.random.uniform(self._next(), shape, jnp.bfloat16, lo, hi)
    def permutation(self, n):
        return jax.random.permutation(self._next(), n)


kernel_name = 'gated_mix__linear_attn_block__glu_gated_swiglu__prompt'

def setup_inputs():
    _rng = _Rng(jax.random.key(int.from_bytes(__import__("os").urandom(4), "little")))
    _w = (lambda a: (lambda t: t.astype(jnp.bfloat16) if jnp.issubdtype(t.dtype, jnp.floating) else t)(jnp.asarray(a)))
    def _A_setup():
        B, S, D = 1, 2048, 1024
        return {
            "x": _w((lambda *s: _rng.normal(s) * 0.05)(B, S, D)),
            "wqkv": _w((lambda *s: _rng.normal(s) * 0.8)(D, 3 * D)),
            "wo": _w((lambda *s: _rng.normal(s) * 0.05)(D, D)),
        }
    _A_in = _A_setup()

    def _B_setup():
        B, S, D, F = 1, 2048, 1024, 3584
        return {
            "x": _w((lambda *s: _rng.normal(s) * 0.05)(B, S, D)),
            "w1": _w((lambda *s: _rng.normal(s) * 1.6)(D, F) * (2.0 / D) ** 0.5),
            "w3": _w((lambda *s: _rng.normal(s) * 1.6)(D, F) * (2.0 / D) ** 0.5),
            "w2": _w((lambda *s: _rng.normal(s) * 1.6)(F, D) * (2.0 / F) ** 0.5),
        }
    _B_in = _B_setup()

    return {
        "A_x": _A_in["x"],
        "A_wqkv": _A_in["wqkv"],
        "A_wo": _A_in["wo"],
        "B_x": _B_in["x"],
        "B_w1": _B_in["w1"],
        "B_w3": _B_in["w3"],
        "B_w2": _B_in["w2"],
        "gate_w": _w((lambda *s: _rng.normal(s) * 0.05)(1024) * 16.0),
    }

def reference(A_x, A_wqkv, A_wo, B_x, B_w1, B_w3, B_w2, gate_w):
    def _A_ref(x, wqkv, wo):
        B, S, D = x.shape
        H = 32; Dh = D // H
        qkv = (lambda x, *d: x.transpose(*d))((x @ wqkv).reshape(B, S, 3, H, Dh), 2, 0, 3, 1, 4)
        q, k, v = qkv[0], qkv[1], qkv[2]
        phi = lambda t: jnp.where(t > 0, t + 1, jnp.exp(t)) + 1e-6
        pq, pk = phi(q), phi(k)
        kv = jnp.einsum("bhsd,bhse->bhde", pk, v)
        z = jnp.einsum("bhsd->bhd", pk)
        num = jnp.einsum("bhqd,bhde->bhqe", pq, kv)
        den = jnp.einsum("bhqd,bhd->bhq", pq, z)[..., None] + 1e-6
        o = num / den
        return (lambda x, *d: x.transpose(*d))(o, 0, 2, 1, 3).reshape(B, S, D) @ wo

    def _B_ref(x, w1, w3, w2):
        gate = jnp.einsum("bsd,df->bsf", x, w1)
        up = jnp.einsum("bsd,df->bsf", x, w3)
        h = _silu(gate) * up
        out = jnp.einsum("bsf,fd->bsd", h, w2)
        return out

    x = A_x
    g = _sigmoid((x * gate_w).sum(-1, keepdims=True))
    a = _A_ref(x, A_wqkv, A_wo)
    b = _B_ref(x, B_w1, B_w3, B_w2)
    return g * a + (1 - g) * b
```

```python
import functools

import jax
import jax.numpy as jnp
import jax.experimental.pallas as pl
import jax.experimental.pallas.tpu as pltpu

F32 = jnp.float32
BF16 = jnp.bfloat16
LANES = 128
NUM_HEADS = 32


def _phi(t):
    return jnp.where(t > 0, t + 1.0, jnp.exp(t)) + 1e-6


def _dot(a, b):
    return jnp.dot(a, b, preferred_element_type=F32)


def _build(S, D, F, *, tm1=512, tn1=512, tm=512, tf=512, tq=512, vmem_mb=100):
    dh = D // NUM_HEADS
    n_t1 = S // tm1
    n_c1 = D // tn1
    n_t2 = S // tm
    n_cf = F // tf
    n_cq = D // tq
    n_g = D // LANES

    def kernel(x_hbm, wqkv_hbm, wo_hbm, w1_hbm, w3_hbm, w2_hbm, gw_ref, out_hbm,
               x_v, wq_v, wk_v, wv_v, wo_v, w1_v, w3_v, w2_v,
               m_v, z_v, kv_acc, z_acc, acc_v, pqn_v, obuf,
               sem_x, sem_q, sem_k, sem_v, sem_o, sem_1, sem_3, sem_2, sem_out):

        def x_copy(i):
            return pltpu.make_async_copy(
                x_hbm.at[0, pl.ds(i * tm1, tm1), :], x_v.at[pl.ds(i * tm1, tm1), :], sem_x.at[i])

        def wq_copy(c):
            return pltpu.make_async_copy(wqkv_hbm.at[:, pl.ds(c * tq, tq)], wq_v.at[c], sem_q.at[c])

        def wk_copy(c):
            return pltpu.make_async_copy(wqkv_hbm.at[:, pl.ds(D + c * tn1, tn1)], wk_v.at[c], sem_k.at[c])

        def wv_copy(c):
            return pltpu.make_async_copy(wqkv_hbm.at[:, pl.ds(2 * D + c * tn1, tn1)], wv_v.at[c], sem_v.at[c])

        def wo_copy():
            return pltpu.make_async_copy(wo_hbm, wo_v, sem_o.at[0])

        def w1_copy(c):
            return pltpu.make_async_copy(w1_hbm.at[:, pl.ds(c * tf, tf)], w1_v.at[c], sem_1.at[c])

        def w3_copy(c):
            return pltpu.make_async_copy(w3_hbm.at[:, pl.ds(c * tf, tf)], w3_v.at[c], sem_3.at[c])

        def w2_copy(c):
            return pltpu.make_async_copy(w2_hbm.at[pl.ds(c * tf, tf), :], w2_v.at[c], sem_2.at[c])

        def out_copy(i, slot):
            return pltpu.make_async_copy(
                obuf.at[slot], out_hbm.at[0, pl.ds(i * tm, tm), :], sem_out.at[slot])

        x_copy(0).start()
        for c in range(n_c1):
            wk_copy(c).start()
            wv_copy(c).start()
        for i in range(1, n_t1):
            x_copy(i).start()
        wo_copy().start()
        for c in range(n_cq):
            wq_copy(c).start()
        for c in range(n_cf):
            w1_copy(c).start()
            w3_copy(c).start()
            w2_copy(c).start()

        kv_acc[...] = jnp.zeros_like(kv_acc)
        z_acc[...] = jnp.zeros_like(z_acc)

        def p1_tile(i, first):
            rows = pl.ds(pl.multiple_of(i * tm1, tm1), tm1)
            xt = x_v[rows, :]
            for c in range(n_c1):
                if first:
                    wk_copy(c).wait()
                    wv_copy(c).wait()
                k = _dot(xt, wk_v[c])
                v = _dot(xt, wv_v[c]).astype(BF16)
                pk = _phi(k)
                pkb = pk.astype(BF16)
                cols = pl.ds(c * tn1, tn1)
                z_acc[:, cols] += jnp.sum(pk.reshape(tm1 // 8, 8, tn1), axis=0)
                for j in range(tn1 // LANES):
                    g = c * (tn1 // LANES) + j
                    sl = slice(j * LANES, (j + 1) * LANES)
                    kv_acc[g] += jax.lax.dot_general(
                        pkb[:, sl], v[:, sl], (((0,), (0,)), ((), ())),
                        preferred_element_type=F32)

        x_copy(0).wait()
        p1_tile(0, True)

        def p1_body(i, carry):
            x_copy(i).wait()
            p1_tile(i, False)
            return carry

        jax.lax.fori_loop(1, n_t1, p1_body, 0)

        wo_copy().wait()
        r = jax.lax.broadcasted_iota(jnp.int32, (LANES, LANES), 0) // dh
        cidx = jax.lax.broadcasted_iota(jnp.int32, (LANES, LANES), 1) // dh
        same_head = r == cidx
        z_row = jnp.sum(z_acc[...], axis=0, keepdims=True)
        for g in range(n_g):
            sl = slice(g * LANES, (g + 1) * LANES)
            kvb = jnp.where(same_head, kv_acc[g], 0.0).astype(BF16)
            m_v[sl, :] = _dot(kvb, wo_v[sl, :]).astype(BF16)
            zt = jnp.broadcast_to(z_row[:, sl], (LANES, LANES)).T
            z_v[g] = jnp.where(same_head, zt, 0.0).astype(BF16)

        for c in range(n_cq):
            wq_copy(c).wait()
        for c in range(n_cf):
            w1_copy(c).wait()
            w3_copy(c).wait()
            w2_copy(c).wait()

        gw = gw_ref[...].astype(F32).reshape(1, D)

        def p2_body(i, carry):
            rows = pl.ds(pl.multiple_of(i * tm, tm), tm)
            xt = x_v[rows, :]
            slot = i % 2

            acc_v[...] = jnp.zeros_like(acc_v)

            def ffn_body(c, carry2):
                gt = _dot(xt, w1_v[c])
                up = _dot(xt, w3_v[c])
                h = (jax.nn.silu(gt) * up).astype(BF16)
                acc_v[...] += _dot(h, w2_v[c])
                return carry2

            jax.lax.fori_loop(0, n_cf, ffn_body, 0)

            for c in range(n_cq):
                q = _dot(xt, wq_v[c])
                pq = _phi(q)
                pqb = pq.astype(BF16)
                for j in range(tq // LANES):
                    g = c * (tq // LANES) + j
                    sl = slice(j * LANES, (j + 1) * LANES)
                    den = _dot(pqb[:, sl], z_v[g]) + 1e-6
                    pqn_v[:, g * LANES:(g + 1) * LANES] = (pq[:, sl] / den).astype(BF16)
            a = _dot(pqn_v[...], m_v[...])

            gs = jnp.sum(xt.astype(F32) * gw, axis=-1, keepdims=True)
            gate = jax.nn.sigmoid(gs)

            @pl.when(i >= 2)
            def _():
                out_copy(i - 2, slot).wait()

            obuf[slot] = (gate * a + (1.0 - gate) * acc_v[...]).astype(BF16)
            out_copy(i, slot).start()
            return carry

        jax.lax.fori_loop(0, n_t2, p2_body, 0)

        for i in range(max(n_t2 - 2, 0), n_t2):
            out_copy(i, i % 2).wait()

    any_spec = pl.BlockSpec(memory_space=pl.ANY)
    scratch = [
        pltpu.VMEM((S, D), BF16),
        pltpu.VMEM((n_cq, D, tq), BF16),
        pltpu.VMEM((n_c1, D, tn1), BF16),
        pltpu.VMEM((n_c1, D, tn1), BF16),
        pltpu.VMEM((D, D), BF16),
        pltpu.VMEM((n_cf, D, tf), BF16),
        pltpu.VMEM((n_cf, D, tf), BF16),
        pltpu.VMEM((n_cf, tf, D), BF16),
        pltpu.VMEM((D, D), BF16),
        pltpu.VMEM((n_g, LANES, LANES), BF16),
        pltpu.VMEM((n_g, LANES, LANES), F32),
        pltpu.VMEM((8, D), F32),
        pltpu.VMEM((tm, D), F32),
        pltpu.VMEM((tm, D), BF16),
        pltpu.VMEM((2, tm, D), BF16),
        pltpu.SemaphoreType.DMA((n_t1,)),
        pltpu.SemaphoreType.DMA((n_cq,)),
        pltpu.SemaphoreType.DMA((n_c1,)),
        pltpu.SemaphoreType.DMA((n_c1,)),
        pltpu.SemaphoreType.DMA((1,)),
        pltpu.SemaphoreType.DMA((n_cf,)),
        pltpu.SemaphoreType.DMA((n_cf,)),
        pltpu.SemaphoreType.DMA((n_cf,)),
        pltpu.SemaphoreType.DMA((2,)),
    ]
    return pl.pallas_call(
        kernel,
        out_shape=jax.ShapeDtypeStruct((1, S, D), BF16),
        in_specs=[any_spec] * 6 + [pl.BlockSpec(memory_space=pltpu.VMEM)],
        out_specs=any_spec,
        scratch_shapes=scratch,
        compiler_params=pltpu.CompilerParams(vmem_limit_bytes=vmem_mb * 1024 * 1024),
    )


@jax.jit
def pallas_gated_mix__linear_attn_block__glu_gated_swiglu__prompt_kernel(
    A_x: jax.Array,
    A_wqkv: jax.Array,
    A_wo: jax.Array,
    B_x: jax.Array,
    B_w1: jax.Array,
    B_w3: jax.Array,
    B_w2: jax.Array,
    gate_w: jax.Array,
):
    del B_x
    _, S, D = A_x.shape
    F = B_w1.shape[1]
    return _build(S, D, F)(A_x, A_wqkv, A_wo, B_w1, B_w3, B_w2, gate_w)
```

```python
import jax
import jax.numpy as jnp
import jax.experimental.pallas as pl
import jax.experimental.pallas.tpu as pltpu

F32 = jnp.float32
BF16 = jnp.bfloat16
LANES = 128
NUM_HEADS = 32


def _phi(t):
    return jnp.where(t > 0, t + 1.0, jnp.exp(t)) + 1e-6


def _dot(a, b):
    return jnp.dot(a, b, preferred_element_type=F32)


def _dot_tn(a, b):
    return jax.lax.dot_general(a, b, (((0,), (0,)), ((), ())), preferred_element_type=F32)


def _dot_nt(a, b):
    return jax.lax.dot_general(a, b, (((1,), (1,)), ((), ())), preferred_element_type=F32)


def _recip(d):
    r0 = pl.reciprocal(d, approx=True)
    return r0 * (2.0 - d * r0)


def _build(S, D, F, *, tm1=256, tm=256, tf=512, tq=512, vmem_mb=100):
    dh = D // NUM_HEADS
    hpg = LANES // dh
    n_t1 = S // tm1
    n_t2 = S // tm
    n_cf = F // tf
    n_cq = D // tq
    n_g = D // LANES
    gpc = tq // LANES

    def kernel(x_hbm, wqkv_hbm, wo_hbm, w1_hbm, w3_hbm, w2_hbm, gw_ref, out_hbm,
               x_v, wq_v, wqt_v, wk_v, wv_v, wo_v, w1_v, w3_v, w2_v, m_v,
               z_v, p_acc, z_acc, ot_v, obuf,
               sem_x, sem_w, sem_1, sem_3, sem_2, sem_out):

        def x_copy(i):
            rows = pl.ds(i * tm1, tm1)
            return pltpu.make_async_copy(x_hbm.at[0, rows, :], x_v.at[rows, :], sem_x.at[i])

        def wq_copy():
            return pltpu.make_async_copy(wqkv_hbm.at[:, pl.ds(0, D)], wq_v, sem_w.at[0])

        def wk_copy():
            return pltpu.make_async_copy(wqkv_hbm.at[:, pl.ds(D, D)], wk_v, sem_w.at[1])

        def wv_copy():
            return pltpu.make_async_copy(wqkv_hbm.at[:, pl.ds(2 * D, D)], wv_v, sem_w.at[2])

        def wo_copy():
            return pltpu.make_async_copy(wo_hbm, wo_v, sem_w.at[3])

        def w1_copy(c):
            return pltpu.make_async_copy(w1_hbm.at[:, pl.ds(c * tf, tf)], w1_v.at[c], sem_1.at[c])

        def w3_copy(c):
            return pltpu.make_async_copy(w3_hbm.at[:, pl.ds(c * tf, tf)], w3_v.at[c], sem_3.at[c])

        def w2_copy(c):
            return pltpu.make_async_copy(w2_hbm.at[pl.ds(c * tf, tf), :], w2_v.at[c], sem_2.at[c])

        def out_copy(i):
            rows = pl.ds(i * tm, tm)
            return pltpu.make_async_copy(obuf.at[rows, :], out_hbm.at[0, rows, :], sem_out.at[i])

        x_copy(0).start()
        wk_copy().start()

        def zero_body(j, carry):
            p_acc[pl.ds(pl.multiple_of(j * 64, 64), 64), :] = jnp.zeros((64, D), F32)
            return carry

        jax.lax.fori_loop(0, D // 64, zero_body, 0)
        z_acc[...] = jnp.zeros_like(z_acc)

        x_copy(0).wait()
        wk_copy().wait()
        for i in range(1, n_t1):
            x_copy(i).start()
        wv_copy().start(priority=1)
        wo_copy().start(priority=1)
        wq_copy().start(priority=1)
        for c in range(n_cf):
            w1_copy(c).start(priority=1)
            w3_copy(c).start(priority=1)
            w2_copy(c).start(priority=1)

        def p1_body(i, carry):
            pl.when(i > 0)(lambda: x_copy(i).wait())
            rows = pl.ds(pl.multiple_of(i * tm1, tm1), tm1)
            k = _dot(x_v[rows, :], wk_v[...])
            xt = x_v[rows, :]
            pk = _phi(k)
            z_acc[...] += jnp.sum(pk.reshape(tm1 // 8, 8, D), axis=0)
            p_acc[...] += _dot_tn(pk.astype(BF16), xt)
            return carry

        jax.lax.fori_loop(0, n_t1, p1_body, 0)

        wv_copy().wait()
        wo_copy().wait()
        wq_copy().wait()
        r = jax.lax.broadcasted_iota(jnp.int32, (LANES, LANES), 0) // dh
        cidx = jax.lax.broadcasted_iota(jnp.int32, (LANES, LANES), 1) // dh
        same_head = r == cidx
        z_row = jnp.sum(z_acc[...], axis=0, keepdims=True)
        for g in range(n_g):
            sl = slice(g * LANES, (g + 1) * LANES)
            kvg = _dot(p_acc[sl, :].astype(BF16), wv_v[:, sl])
            kvb = jnp.where(same_head, kvg, 0.0).astype(BF16)
            m_v[sl, :] = _dot(kvb, wo_v[sl, :]).astype(BF16)
            z_v[g] = jnp.broadcast_to(z_row[:, sl], (LANES, LANES)).T
            wqt_v[sl, :] = wq_v[:, sl].T

        for c in range(n_cf):
            w1_copy(c).wait()
            w3_copy(c).wait()
            w2_copy(c).wait()

        gw = gw_ref[...].astype(F32).reshape(1, D)

        def p2_body(i, carry):
            rows = pl.ds(pl.multiple_of(i * tm, tm), tm)
            xt = x_v[rows, :]

            for c in range(n_cq):
                qt = _dot_nt(wqt_v[c * tq:(c + 1) * tq, :], xt)
                for j in range(gpc):
                    g = c * gpc + j
                    pq = _phi(qt[j * LANES:(j + 1) * LANES, :])
                    zc = jnp.concatenate([z_v[g]] * (tm // LANES), axis=1)
                    den = jnp.sum((pq * zc).reshape(hpg, dh, tm), axis=1, keepdims=True) + 1e-6
                    o = pq.reshape(hpg, dh, tm) * _recip(den)
                    ot_v[g * LANES:(g + 1) * LANES, :] = o.reshape(LANES, tm).astype(BF16)

            b = None
            for c in range(n_cf):
                gt = _dot(xt, w1_v[c])
                up = _dot(xt, w3_v[c])
                h = (jax.nn.silu(gt) * up).astype(BF16)
                d = _dot(h, w2_v[c])
                b = d if b is None else b + d

            a = _dot_tn(ot_v[...], m_v[...])

            gate = jax.nn.sigmoid(jnp.sum(xt.astype(F32) * gw, axis=-1, keepdims=True))
            obuf[rows, :] = (gate * a + (1.0 - gate) * b).astype(BF16)
            out_copy(i).start()
            return carry

        jax.lax.fori_loop(0, n_t2, p2_body, 0)

        for i in range(n_t2):
            out_copy(i).wait()

    any_spec = pl.BlockSpec(memory_space=pl.ANY)
    scratch = [
        pltpu.VMEM((S, D), BF16),
        pltpu.VMEM((D, D), BF16),
        pltpu.VMEM((D, D), BF16),
        pltpu.VMEM((D, D), BF16),
        pltpu.VMEM((D, D), BF16),
        pltpu.VMEM((D, D), BF16),
        pltpu.VMEM((n_cf, D, tf), BF16),
        pltpu.VMEM((n_cf, D, tf), BF16),
        pltpu.VMEM((n_cf, tf, D), BF16),
        pltpu.VMEM((D, D), BF16),
        pltpu.VMEM((n_g, LANES, LANES), F32),
        pltpu.VMEM((D, D), F32),
        pltpu.VMEM((8, D), F32),
        pltpu.VMEM((D, tm), BF16),
        pltpu.VMEM((S, D), BF16),
        pltpu.SemaphoreType.DMA((n_t1,)),
        pltpu.SemaphoreType.DMA((4,)),
        pltpu.SemaphoreType.DMA((n_cf,)),
        pltpu.SemaphoreType.DMA((n_cf,)),
        pltpu.SemaphoreType.DMA((n_cf,)),
        pltpu.SemaphoreType.DMA((n_t2,)),
    ]
    return pl.pallas_call(
        kernel,
        out_shape=jax.ShapeDtypeStruct((1, S, D), BF16),
        in_specs=[any_spec] * 6 + [pl.BlockSpec(memory_space=pltpu.VMEM)],
        out_specs=any_spec,
        scratch_shapes=scratch,
        compiler_params=pltpu.CompilerParams(vmem_limit_bytes=vmem_mb * 1024 * 1024),
    )


@jax.jit
def pallas_gated_mix__linear_attn_block__glu_gated_swiglu__prompt_kernel(
    A_x: jax.Array,
    A_wqkv: jax.Array,
    A_wo: jax.Array,
    B_x: jax.Array,
    B_w1: jax.Array,
    B_w3: jax.Array,
    B_w2: jax.Array,
    gate_w: jax.Array,
):
    del B_x
    _, S, D = A_x.shape
    F = B_w1.shape[1]
    return _build(S, D, F)(A_x, A_wqkv, A_wo, B_w1, B_w3, B_w2, gate_w)
```

```python
import jax
import jax.numpy as jnp
import jax.experimental.pallas as pl
import jax.experimental.pallas.tpu as pltpu

F32 = jnp.float32
BF16 = jnp.bfloat16
LANES = 128
NUM_HEADS = 32

ROWS1 = 256
ROWS2 = 256
K_CHUNKS = (256, 256, 512)
OUT_SPLIT = 8
LOW = 1


def _phi(t):
    return jnp.where(t > 0, t + 1.0, jnp.exp(t)) + 1e-6


def _dot(a, b):
    return jnp.dot(a, b, preferred_element_type=F32)


def _dot_tn(a, b):
    return jax.lax.dot_general(a, b, (((0,), (0,)), ((), ())), preferred_element_type=F32)


def _dot_nt(a, b):
    return jax.lax.dot_general(a, b, (((1,), (1,)), ((), ())), preferred_element_type=F32)


def _reciprocal(d):
    r = pl.reciprocal(d, approx=True)
    return r * (2.0 - d * r)


def _build(S, D, F, *, vmem_mb=100):
    dh = D // NUM_HEADS
    hpg = LANES // dh
    n_g = D // LANES
    n_t1 = S // ROWS1
    n_t2 = S // ROWS2
    k_off = [sum(K_CHUNKS[:c]) for c in range(len(K_CHUNKS))]
    ow = D // OUT_SPLIT
    assert sum(K_CHUNKS) == D and len(K_CHUNKS) == 3
    assert S % ROWS1 == 0 and S % ROWS2 == 0 and LANES % dh == 0

    def kernel(x_hbm, wqkv_hbm, wo_hbm, w1_hbm, w3_hbm, w2_hbm, gw_ref, out_hbm,
               x_v, wq_v, wqt_v, wk_v, wv_v, wo_v, w1_v, w3_v, w2_v, m_v,
               z_v, p_acc, z_acc, ot_v, obuf,
               sem_x, sem_k, sem_mid, sem_ffn, sem_out):

        def x_copy(i):
            rows = pl.ds(i * ROWS1, ROWS1)
            return pltpu.make_async_copy(x_hbm.at[0, rows, :], x_v.at[rows, :], sem_x.at[i])

        def wk_copy(c):
            return pltpu.make_async_copy(
                wqkv_hbm.at[:, pl.ds(D + k_off[c], K_CHUNKS[c])],
                wk_v.at[:, pl.ds(k_off[c], K_CHUNKS[c])], sem_k.at[c])

        mid_copies = [
            pltpu.make_async_copy(wqkv_hbm.at[:, pl.ds(2 * D, D)], wv_v, sem_mid),
            pltpu.make_async_copy(wo_hbm, wo_v, sem_mid),
            pltpu.make_async_copy(wqkv_hbm.at[:, pl.ds(0, D)], wq_v, sem_mid),
        ]
        ffn_copies = [
            pltpu.make_async_copy(w1_hbm, w1_v, sem_ffn),
            pltpu.make_async_copy(w3_hbm, w3_v, sem_ffn),
            pltpu.make_async_copy(w2_hbm, w2_v, sem_ffn),
        ]

        def k_chunk(c):
            return _dot(x_v[0:ROWS1, :], wk_v[:, k_off[c]:k_off[c] + K_CHUNKS[c]])

        def p_chunk(c, k):
            cols = slice(k_off[c], k_off[c] + K_CHUNKS[c])
            pk = _phi(k)
            z_acc[:, cols] = jnp.sum(pk.reshape(ROWS1 // 8, 8, K_CHUNKS[c]), axis=0)
            p_acc[cols, :] = _dot_tn(pk.astype(BF16), x_v[0:ROWS1, :])

        x_copy(0).start()
        wk_copy(0).start()
        wk_copy(1).start(priority=LOW)

        x_copy(0).wait()
        wk_copy(0).wait()
        wk_copy(2).start(priority=LOW)
        k0 = k_chunk(0)

        wk_copy(1).wait()
        k1 = k_chunk(1)
        p_chunk(0, k0)

        wk_copy(2).wait()
        for i in range(1, n_t1):
            x_copy(i).start()
        for cp in mid_copies + ffn_copies:
            cp.start(priority=LOW)
        k2 = k_chunk(2)
        p_chunk(1, k1)
        p_chunk(2, k2)

        def p1_body(i, carry):
            x_copy(i).wait()
            rows = pl.ds(pl.multiple_of(i * ROWS1, ROWS1), ROWS1)
            k = _dot(x_v[rows, :], wk_v[...])
            xt = x_v[rows, :]
            pk = _phi(k)
            z_acc[...] += jnp.sum(pk.reshape(ROWS1 // 8, 8, D), axis=0)
            p_acc[...] += _dot_tn(pk.astype(BF16), xt)
            return carry

        jax.lax.fori_loop(1, n_t1, p1_body, 0)

        for cp in mid_copies:
            cp.wait()
        row_head = jax.lax.broadcasted_iota(jnp.int32, (LANES, LANES), 0) // dh
        col_head = jax.lax.broadcasted_iota(jnp.int32, (LANES, LANES), 1) // dh
        same_head = row_head == col_head
        z_row = jnp.sum(z_acc[...], axis=0, keepdims=True)
        gw = gw_ref[...].astype(F32).reshape(1, D)
        kv_blocks = []
        for g in range(n_g):
            sl = slice(g * LANES, (g + 1) * LANES)
            kv = _dot(p_acc[sl, :].astype(BF16), wv_v[:, sl])
            kv_blocks.append(jnp.where(same_head, kv, 0.0).astype(BF16))
        for g in range(n_g):
            sl = slice(g * LANES, (g + 1) * LANES)
            m_v[sl, :] = _dot(kv_blocks[g], wo_v[sl, :]).astype(BF16)
            z_v[g] = jnp.broadcast_to(z_row[:, sl], (LANES, LANES)).T
            wqt_v[sl, :] = wq_v[:, sl].T

        for cp in ffn_copies:
            cp.wait()

        def p2_body(i, carry):
            rows = pl.ds(pl.multiple_of(i * ROWS2, ROWS2), ROWS2)
            xt = x_v[rows, :]

            gate_act = _dot(xt, w1_v[...])
            up = _dot(xt, w3_v[...])
            h = (jax.nn.silu(gate_act) * up).astype(BF16)

            qt = _dot_nt(wqt_v[...], xt)
            for g in range(n_g):
                pq = _phi(qt[g * LANES:(g + 1) * LANES, :])
                zc = jnp.concatenate([z_v[g]] * (ROWS2 // LANES), axis=1)
                den = jnp.sum((pq * zc).reshape(hpg, dh, ROWS2), axis=1, keepdims=True) + 1e-6
                o = pq.reshape(hpg, dh, ROWS2) * _reciprocal(den)
                ot_v[g * LANES:(g + 1) * LANES, :] = o.reshape(LANES, ROWS2).astype(BF16)

            gate = jax.nn.sigmoid(jnp.sum(xt.astype(F32) * gw, axis=-1, keepdims=True))
            a = _dot_tn(ot_v[...], m_v[...])

            for s in range(OUT_SPLIT):
                cs = slice(s * ow, (s + 1) * ow)
                b = _dot(h, w2_v[:, cs])
                obuf[rows, cs] = (gate * a[:, cs] + (1.0 - gate) * b).astype(BF16)
                pltpu.make_async_copy(
                    obuf.at[rows, pl.ds(s * ow, ow)],
                    out_hbm.at[0, rows, pl.ds(s * ow, ow)], sem_out).start()
            return carry

        jax.lax.fori_loop(0, n_t2, p2_body, 0)

        pltpu.make_async_copy(obuf, out_hbm.at[0], sem_out).wait()

    any_spec = pl.BlockSpec(memory_space=pl.ANY)
    scratch = [
        pltpu.VMEM((S, D), BF16),
        pltpu.VMEM((D, D), BF16),
        pltpu.VMEM((D, D), BF16),
        pltpu.VMEM((D, D), BF16),
        pltpu.VMEM((D, D), BF16),
        pltpu.VMEM((D, D), BF16),
        pltpu.VMEM((D, F), BF16),
        pltpu.VMEM((D, F), BF16),
        pltpu.VMEM((F, D), BF16),
        pltpu.VMEM((D, D), BF16),
        pltpu.VMEM((n_g, LANES, LANES), F32),
        pltpu.VMEM((D, D), F32),
        pltpu.VMEM((8, D), F32),
        pltpu.VMEM((D, ROWS2), BF16),
        pltpu.VMEM((S, D), BF16),
        pltpu.SemaphoreType.DMA((n_t1,)),
        pltpu.SemaphoreType.DMA((len(K_CHUNKS),)),
        pltpu.SemaphoreType.DMA(()),
        pltpu.SemaphoreType.DMA(()),
        pltpu.SemaphoreType.DMA(()),
    ]
    return pl.pallas_call(
        kernel,
        out_shape=jax.ShapeDtypeStruct((1, S, D), BF16),
        in_specs=[any_spec] * 6 + [pl.BlockSpec(memory_space=pltpu.VMEM)],
        out_specs=any_spec,
        scratch_shapes=scratch,
        compiler_params=pltpu.CompilerParams(vmem_limit_bytes=vmem_mb * 1024 * 1024),
    )


@jax.jit
def pallas_gated_mix__linear_attn_block__glu_gated_swiglu__prompt_kernel(
    A_x: jax.Array,
    A_wqkv: jax.Array,
    A_wo: jax.Array,
    B_x: jax.Array,
    B_w1: jax.Array,
    B_w3: jax.Array,
    B_w2: jax.Array,
    gate_w: jax.Array,
):
    del B_x
    _, S, D = A_x.shape
    F = B_w1.shape[1]
    return _build(S, D, F)(A_x, A_wqkv, A_wo, B_w1, B_w3, B_w2, gate_w)
```
